```python
import jax
import jax.numpy as jnp

def _softmax(x, axis=-1):
    return jax.nn.softmax(x, axis=axis)
def _gelu(x):
    return jax.nn.gelu(x, approximate=True)
def _silu(x):
    return jax.nn.silu(x)
def _sigmoid(x):
    return jax.nn.sigmoid(x)
def _layernorm(x, axis=-1, eps=1e-5):
    m = jnp.mean(x, axis=axis, keepdims=True)
    v = jnp.var(x, axis=axis, keepdims=True)
    return (x - m) / jnp.sqrt(v + eps)
def _scatter_add(tgt, idx, src, axis=0):
    return tgt.at[idx].add(src)
def _segment_sum(src, seg, n):
    return jax.ops.segment_sum(src, seg, n)
class _Rng:
    def __init__(self, key):
        self._k = key
    def _next(self):
        self._k, sub = jax.random.split(self._k)
        return sub
    def normal(self, shape):
        return jax.random.normal(self._next(), shape, dtype=jnp.bfloat16)
    def randint(self, lo, hi, shape):
        return jax.random.randint(self._next(), shape, lo, hi, dtype=jnp.int32)
    def uniform(self, shape, lo=0.0, hi=1.0):
        return jax.random.uniform(self._next(), shape, jnp.bfloat16, lo, hi)
    def permutation(self, n):
        return jax.random.permutation(self._next(), n)


kernel_name = 'sequential_preLN__sliding_block__glu_gated_glu__prompt'

def _fwd_setup_inputs():
    _rng = _Rng(jax.random.key(int.from_bytes(__import__("os").urandom(4), "little")))
    _w = (lambda a: (lambda t: t.astype(jnp.bfloat16) if jnp.issubdtype(t.dtype, jnp.floating) else t)(jnp.asarray(a)))
    def _A_setup():
        B, S, D = 1, 2048, 512
        return {
            "x": _w((lambda *s: _rng.normal(s) * 0.05)(B, S, D)),
            "wqkv": _w((lambda *s: _rng.normal(s) * 0.05)(D, 3 * D)),
            "wo": _w((lambda *s: _rng.normal(s) * 0.05)(D, D)),
        }
    _A_in = _A_setup()

    def _B_setup():
        B, S, D, F = 1, 2048, 512, 1376
        return {
            "x": _w((lambda *s: _rng.normal(s) * 0.05)(B, S, D)),
            "w_gate": _w((lambda *s: _rng.normal(s) * 0.05)(D, F)),
            "w_up": _w((lambda *s: _rng.normal(s) * 0.05)(D, F)),
            "w_down": _w((lambda *s: _rng.normal(s) * 0.05)(F, D)),
        }
    _B_in = _B_setup()

    return {
        "A_x": _A_in["x"],
        "A_wqkv": _A_in["wqkv"],
        "A_wo": _A_in["wo"],
        "B_x": _B_in["x"],
        "B_w_gate": _B_in["w_gate"],
        "B_w_up": _B_in["w_up"],
        "B_w_down": _B_in["w_down"],
    }

def _fwd_reference(A_x, A_wqkv, A_wo, B_x, B_w_gate, B_w_up, B_w_down):
    def _A_ref(x, wqkv, wo):
        B, S, D = x.shape
        H = 32; Dh = D // H; W = 256
        qkv = (lambda x, *d: x.transpose(*d))((x @ wqkv).reshape(B, S, 3, H, Dh), 2, 0, 3, 1, 4)
        q, k, v = qkv[0], qkv[1], qkv[2]
        scores = jnp.einsum("bhqd,bhkd->bhqk", q, k) * (Dh ** -0.5)
        idx = jnp.arange(S)
        mask = (idx[:, None] - idx[None, :] >= 0) & (idx[:, None] - idx[None, :] < W)
        scores = jnp.where(mask[None, None], scores, -1e9)
        p = _softmax(scores, axis=-1)
        o = jnp.einsum("bhqk,bhkd->bhqd", p, v)
        return (lambda x, *d: x.transpose(*d))(o, 0, 2, 1, 3).reshape(B, S, D) @ wo

    def _B_ref(x, w_gate, w_up, w_down):
        g = jnp.einsum("bsd,df->bsf", x, w_gate)
        u = jnp.einsum("bsd,df->bsf", x, w_up)
        h = _sigmoid(g) * u
        return jnp.einsum("bsf,fd->bsd", h, w_down)

    x = A_x
    h = x + _A_ref(_layernorm(x, axis=-1), A_wqkv, A_wo)
    h2 = h + _B_ref(_layernorm(h, axis=-1), B_w_gate, B_w_up, B_w_down)
    return h2


def setup_inputs():
    _inp = _fwd_setup_inputs()
    _gk = jax.random.fold_in(jax.random.key(int.from_bytes(__import__("os").urandom(4), "little")), 2**31 - 1)
    _shapes = [[1, 2048, 512]]
    _dtypes = ['bfloat16']
    _gks = jax.random.split(_gk, len(_shapes))
    _gs = [jax.random.normal(k, s, dtype=jnp.dtype(d)) * 0.05 for k, s, d in zip(_gks, _shapes, _dtypes)]
    _inp["grad_out"] = _gs[0]
    return _inp

def reference(A_x, A_wqkv, A_wo, B_w_gate, B_w_up, B_w_down, B_x, grad_out):
    _const = dict(B_x=B_x)
    def _f(*_d):
        return _fwd_reference(**{'A_x': _d[0], 'A_wqkv': _d[1], 'A_wo': _d[2], 'B_w_gate': _d[3], 'B_w_up': _d[4], 'B_w_down': _d[5], **_const})
    _out, _vjp = jax.vjp(_f, A_x, A_wqkv, A_wo, B_w_gate, B_w_up, B_w_down)
    _grads = _vjp(grad_out)
    _out0 = jnp.asarray(_out)
    return (_out0, *[jnp.asarray(_g) for _g in _grads])
```

```python
import jax
import jax.numpy as jnp
from jax import lax
import jax.experimental.pallas as pl
import jax.experimental.pallas.tpu as pltpu

S, D, F = 2048, 512, 1376
W = 256
T = 256
NB = S // T
QB = T // 128
G = 4
NK0 = (S + W) // 128
BWD_ORDER = ((0, 0), (3, 1), (1, 1), (2, 2))
EPS = 1e-5
F32, BF16 = jnp.float32, jnp.bfloat16
FCH = ((0, 384), (384, 384), (768, 256), (1024, 352))


def _nn(a, b):
    return jnp.dot(a, b, preferred_element_type=F32)


def _nt(a, b):
    return lax.dot_general(a, b, (((1,), (1,)), ((), ())), preferred_element_type=F32)


def _tn(a, b):
    return lax.dot_general(a, b, (((0,), (0,)), ((), ())), preferred_element_type=F32)


class _Pk:
    def __init__(self, ref):
        self.ref = ref

    def _ix(self, ix):
        ix = ix if isinstance(ix, tuple) else (ix,)
        if len(ix) == len(self.ref.shape) - 1:
            r = ix[-1]
            if isinstance(r, slice):
                r = slice(r.start // 2, r.stop // 2)
            else:
                st = r.start // 2
                r = pl.ds(st if isinstance(st, int) else pl.multiple_of(st, 8), r.size // 2)
            ix = ix[:-1] + (r,)
        return ix

    def __getitem__(self, ix):
        return pltpu.bitcast(self.ref[self._ix(ix)], BF16)

    def __setitem__(self, ix, v):
        self.ref[self._ix(ix)] = pltpu.bitcast(v, jnp.int32)


def _ln(x):
    m = jnp.mean(x, axis=-1, keepdims=True)
    xc = x - m
    v = jnp.mean(xc * xc, axis=-1, keepdims=True)
    r = 1.0 / jnp.sqrt(v + EPS)
    return xc * r, r


def _ln_bwd(dy, y, r):
    return r * (dy - jnp.mean(dy, axis=-1, keepdims=True)
                - y * jnp.mean(dy * y, axis=-1, keepdims=True))


def _roll_odd(t):
    parts = []
    for h in range(8):
        p = t[16 * h:16 * h + 16]
        parts.append(pltpu.roll(p, 64, 1) if h % 2 else p)
    return jnp.concatenate(parts, axis=0)


def kernel(x_h, wqkv_h, wo_h, wg_h, wu_h, wd_h, go_h,
           out_h, dx_h, dwqkv_h, dwo_h, dwg_h, dwu_h, dwd_h,
           x_ref, wqkv_ref, wo_ref, wg_ref, wu_ref, wd_ref, go_ref,
           out_ref, dx_ref, dwqkv_ref, dwo_ref, dwg_ref, dwu_ref, dwd_ref, isem, osem, rsem,
           q_s, k_s, v_s, qt_s, kt_s, vt_s, p_s, il_s, ot_s, do_s, dot_s, dl_s,
           dh_s, dqt_s, dkt_s, dvt_s, awqkv, awo, awg, awu, awd):
    ins = [pltpu.make_async_copy(a, d, isem.at[i]) for i, (a, d) in enumerate((
        (x_h.at[0:T], x_ref.at[0:T]), (wqkv_h, wqkv_ref), (x_h.at[T:S], x_ref.at[T:S]),
        (wo_h, wo_ref), (wg_h, wg_ref), (wu_h, wu_ref), (go_h, go_ref), (wd_h, wd_ref)))]
    outs = [pltpu.make_async_copy(a, d, osem.at[i]) for i, (a, d) in enumerate((
        (dwo_ref, dwo_h), (dwg_ref, dwg_h), (dwu_ref, dwu_h), (dwd_ref, dwd_h), (dwqkv_ref, dwqkv_h)))]

    def row_copy(k, b):
        src, dst = ((out_ref, out_h), (dx_ref, dx_h))[k]
        rows = pl.ds(pl.multiple_of(b * T, T), T)
        return pltpu.make_async_copy(src.at[rows], dst.at[rows], rsem.at[k, b])
    for c in ins:
        c.start()
    q_s, k_s, v_s, kt_s, vt_s, p_s, do_s = map(
        _Pk, (q_s, k_s, v_s, kt_s, vt_s, p_s, do_s))
    lane = lax.broadcasted_iota(jnp.int32, (64, 128), 1)
    row = lax.broadcasted_iota(jnp.int32, (64, 128), 0)
    diag = row <= (lane & 63)
    lo16 = lax.broadcasted_iota(jnp.int32, (16, 128), 1) < 64
    lo1 = lax.broadcasted_iota(jnp.int32, (1, 128), 1) < 64
    z64 = jnp.zeros((64, 128), BF16)

    for g in range(G):
        q_s[g, S:S + W] = jnp.zeros((W, 128), BF16)
        k_s[g, S + W:S + 2 * W] = jnp.zeros((W, 128), BF16)
        for j in range(2):
            vt_s[g, NK0 + j] = jnp.zeros((128, 128), BF16)
        k_s[g, 0:W] = jnp.zeros((W, 128), BF16)
        v_s[g, 0:W] = jnp.zeros((W, 128), BF16)
        for j in range(2):
            kt_s[g, j] = jnp.zeros((128, 128), BF16)
            vt_s[g, j] = jnp.zeros((128, 128), BF16)
        for j in range(2):
            dkt_s[g, j] = jnp.zeros((128, 128), F32)
            dvt_s[g, j] = jnp.zeros((128, 128), F32)

    awo[...] = jnp.zeros_like(awo)
    awg[...] = jnp.zeros_like(awg)
    awu[...] = jnp.zeros_like(awu)
    awd[...] = jnp.zeros_like(awd)
    awqkv[...] = jnp.zeros_like(awqkv)
    ins[0].wait()
    ins[1].wait()

    def p1(b, side):
        @pl.when(b == 1)
        def _():
            ins[2].wait()
        r0 = pl.multiple_of(b * T, T)
        side()
        y, r = _ln(x_ref[pl.ds(r0, T)].astype(F32))
        yb = y.astype(BF16)
        side()
        for i, (ns, ts) in enumerate(((q_s, qt_s), (k_s, kt_s), (v_s, vt_s))):
            z = _nn(yb, wqkv_ref[:, i * D:(i + 1) * D])
            if i < 2:
                side()
            if i == 0:
                z = z * 0.25
            off = 0 if i == 0 else W
            for g in range(G):
                zg = z[:, g * 128:(g + 1) * 128]
                ns[g, pl.ds(r0 + off, T)] = zg.astype(BF16)
                for j in range(QB):
                    zt = zg[j * 128:(j + 1) * 128].T
                    if i == 0:
                        zt = _roll_odd(zt)
                    ts[g, b * QB + j + off // 128] = zt if i == 0 else zt.astype(BF16)

    def headmask(h):
        return (lane >= 16 * h) & (lane < 16 * h + 16)

    def bd_nat(t, a, b):
        te, to = t[0:64], t[64:128]
        zz = jnp.zeros_like(te)
        e = jnp.concatenate([jnp.where(headmask(a), te, zz), jnp.where(headmask(b), te, zz)], 0)
        o = jnp.concatenate([jnp.where(headmask(b), to, zz), jnp.where(headmask(a), to, zz)], 0)
        return e, o

    def bd_t(ta, tb):
        zz = jnp.zeros_like(ta)
        e = jnp.concatenate([jnp.where(lo16, ta, zz), jnp.where(lo16, zz, tb)], 0)
        o = jnp.concatenate([jnp.where(lo16, zz, ta), jnp.where(lo16, tb, zz)], 0)
        return e, o

    def softmax_t(s, kbase):
        sm = jnp.where(diag, s[256:320], s[0:64])
        mid = s[64:256]
        if kbase is not None:
            sm = jnp.where(diag | (kbase >= 0), sm, -1e30)
            mid = jnp.concatenate(
                [jnp.where(kbase + 64 * (c + 1) >= 0, mid[64 * c:64 * c + 64], -1e30)
                 for c in range(3)], 0)
        m = jnp.maximum(jnp.max(sm, axis=0, keepdims=True), jnp.max(mid, axis=0, keepdims=True))
        em = jnp.exp(sm - m)
        emid = jnp.exp(mid - m)
        inv = 1.0 / (jnp.sum(em, axis=0, keepdims=True) + jnp.sum(emid, axis=0, keepdims=True))
        return jnp.concatenate([jnp.where(diag, 0.0, em).astype(BF16), emid.astype(BF16),
                                jnp.where(diag, em, 0.0).astype(BF16)], 0), inv

    def attn_fwd(b, j, g, edge):
        qb = b * QB + j
        pj = (b % 2) * QB + j
        q0 = pl.multiple_of(qb * 128, 128)
        sc = {}
        def A(p):
            qe, qo = bd_nat(q_s[g, pl.ds(q0, 128)], 2 * p, 2 * p + 1)
            sc[p] = (_nt(k_s[g, pl.ds(q0, 320)], qe), _nt(k_s[g, pl.ds(q0 + 64, 320)], qo))
        def B(p):
            pe, ie = softmax_t(sc[p][0], (q0 - W) if edge else None)
            po, io = softmax_t(sc[p][1], (q0 - W + 64) if edge else None)
            p_s[pj, g, 2 * p] = pe
            il_s[qb, g, 2 * p:2 * p + 1] = jnp.where(lo1, ie, io)
            il_s[qb, g, 2 * p + 1:2 * p + 2] = jnp.where(lo1, io, ie)
            p_s[pj, g, 2 * p + 1] = po
            sc[p] = pe, po, ie, io
        def C(p):
            ia = il_s[qb, g, 2 * p:2 * p + 1]
            ib = il_s[qb, g, 2 * p + 1:2 * p + 2]
            pe, po, ie, io = sc[p]
            vt = jnp.concatenate([vt_s[g, qb + c, 32 * p:32 * p + 32] for c in range(3)], 1)
            oe = _nn(vt, jnp.concatenate([pe, z64], 0)) * ie
            oo = _nn(vt, jnp.concatenate([z64, po], 0)) * io
            ot_s[g, qb, 32 * p:32 * p + 16] = jnp.where(lo16, oe[0:16], oo[0:16])
            ot_s[g, qb, 32 * p + 16:32 * p + 32] = pltpu.roll(
                jnp.where(lo16, oo[16:32], oe[16:32]), 64, 1)
        return [lambda: A(0), lambda: A(1), lambda: B(0), lambda: A(2), lambda: (B(1), C(0)),
                lambda: A(3), lambda: (B(2), C(1)), lambda: (B(3), C(2), C(3))]

    def kv_grad(acc, g, qb, p, le, lo, pe, po):
        rs = slice(32 * p, 32 * p + 32)
        t0 = _nt(le, pe[0:128])
        t1 = _nt(le, pe[128:256]) + _nt(lo, po[64:192])
        t2 = _nt(lo, po[192:320])
        tm = _nt(jnp.concatenate([le, lo], 0), jnp.concatenate([pe[256:320], po[0:64]], 0))
        lo32 = lax.broadcasted_iota(jnp.int32, (32, 128), 1) < 64
        acc[g, qb, rs] += t0 + jnp.where(lo32, 0.0, tm[32:64])
        acc[g, qb + 1, rs] += t1
        acc[g, qb + 2, rs] = t2 + jnp.where(lo32, tm[0:32], 0.0)

    def attn_bwd(b, j, g):
        qb = b * QB + j
        q0 = pl.multiple_of(qb * 128, 128)
        pj = (b % 2) * QB + j
        dot_ = do_s[g, pl.ds(j * 128, 128)]
        sc = {}
        def A(p):
            de, do = bd_nat(dot_, 2 * p, 2 * p + 1)
            sc[p] = _nt(v_s[g, pl.ds(q0, 320)], de), _nt(v_s[g, pl.ds(q0 + 64, 320)], do)
        def B(p):
            ia = il_s[qb, g, 2 * p:2 * p + 1]
            ib = il_s[qb, g, 2 * p + 1:2 * p + 2]
            da = dl_s[g, j, 2 * p:2 * p + 1]
            db = dl_s[g, j, 2 * p + 1:2 * p + 2]
            pe = p_s[pj, g, 2 * p]
            po = p_s[pj, g, 2 * p + 1]
            se = (pe.astype(F32) * (sc[p][0] - jnp.where(lo1, da, db))).astype(BF16)
            so = (po.astype(F32) * (sc[p][1] - jnp.where(lo1, db, da))).astype(BF16)
            sc[p] = se, so
        def V(p):
            ia = il_s[qb, g, 2 * p:2 * p + 1]
            ib = il_s[qb, g, 2 * p + 1:2 * p + 2]
            ra = slice(32 * p, 32 * p + 16)
            rb = slice(32 * p + 16, 32 * p + 32)
            le, lo = bd_t((dot_s[g, j, ra] * ia).astype(BF16), (dot_s[g, j, rb] * ib).astype(BF16))
            kv_grad(dvt_s, g, qb, p, le, lo, p_s[pj, g, 2 * p], p_s[pj, g, 2 * p + 1])
        def C(p):
            ia = il_s[qb, g, 2 * p:2 * p + 1]
            ib = il_s[qb, g, 2 * p + 1:2 * p + 2]
            rs = slice(32 * p, 32 * p + 32)
            ra = slice(32 * p, 32 * p + 16)
            rb = slice(32 * p + 16, 32 * p + 32)
            se, so = sc[p]
            kt = jnp.concatenate([kt_s[g, qb + c, rs] for c in range(3)], 1)
            qe_ = _nn(kt, jnp.concatenate([se, z64], 0))
            qo_ = _nn(kt, jnp.concatenate([z64, so], 0))
            dqt_s[g, qb, ra] = jnp.where(lo16, qe_[0:16], qo_[0:16]) * ia
            dqt_s[g, qb, rb] = pltpu.roll(jnp.where(lo16, qo_[16:32], qe_[16:32]) * ib, 64, 1)
            le, lo = bd_t((qt_s[g, qb, ra] * ia).astype(BF16), (qt_s[g, qb, rb] * ib).astype(BF16))
            kv_grad(dkt_s, g, qb, p, le, lo, se, so)
        return A, B, C, V

    def mlp(b):
        r0 = pl.multiple_of(b * T, T)
        z = b // 64
        steps = iter([st for j in range(QB) for g in range(G)
                      for st in attn_fwd(b + 1, j + z, g + z, False)])

        def side(n=2):
            for _ in range(n):
                next(steps)()
        side(2)
        das = [_nt(go_ref[pl.ds(r0, T)], wd_ref[0:FCH[0][1], :])]
        otb = jnp.concatenate(
            [jnp.concatenate([ot_s[g, b * QB + j] for j in range(QB)], 1) for g in range(G)], 0)
        otb16 = otb.astype(BF16)
        h = x_ref[pl.ds(r0, T)].astype(F32) + _tn(otb16, wo_ref[...])
        side(2)
        das.append(_nt(go_ref[pl.ds(r0, T)], wd_ref[FCH[1][0]:FCH[2][0], :]))
        y, r = _ln(h)
        side(2)
        das.append(_nt(go_ref[pl.ds(r0, T)], wd_ref[FCH[2][0]:FCH[3][0], :]))
        yb = y.astype(BF16)
        go = go_ref[pl.ds(r0, T)]
        out = h
        dy = jnp.zeros((T, D), F32)
        side(2)
        for ci, (f0, fn) in enumerate(FCH):
            last = ci == len(FCH) - 1
            fs = slice(f0, f0 + fn)
            wg, wu, wd = wg_ref[fs, :], wu_ref[fs, :], wd_ref[fs, :]
            da = das[ci] if ci < 3 else _nt(go, wd)
            side()
            sg = jax.nn.sigmoid(_nt(yb, wg))
            side()
            u = _nt(yb, wu)
            side()
            a = (sg * u).astype(BF16)
            du32 = da * sg
            du = du32.astype(BF16)
            dg = (du32 * u * (1.0 - sg)).astype(BF16)
            out = out + _nn(a, wd)
            side()
            dy = dy + _nn(dg, wg) + _nn(du, wu)
            side()
            if last:
                out_ref[pl.ds(r0, T)] = out.astype(BF16)
                dh = go.astype(F32) + _ln_bwd(dy, y, r)
            awd[fs, :] += _tn(a, go)
            if not last:
                side()
                awg[fs, :] += _tn(dg, yb)
                side()
                awu[fs, :] += _tn(du, yb)
        dh_s[pl.ds(r0, T)] = dh
        dhb = dh.astype(BF16)
        do = _nt(dhb, wo_ref[...])
        for g in range(G):
            dg_ = do[:, g * 128:(g + 1) * 128]
            do_s[g] = dg_.astype(BF16)
            for j in range(QB):
                t = _roll_odd(dg_[j * 128:(j + 1) * 128].T)
                dot_s[g, j] = t
                pr = t * _roll_odd(ot_s[g, b * QB + j])
                for hh in range(8):
                    dl_s[g, j, hh:hh + 1] = jnp.sum(pr[16 * hh:16 * hh + 16], axis=0, keepdims=True)
        side()
        awg[fs, :] += _tn(dg, yb)
        side()
        awu[fs, :] += _tn(du, yb)
        awo[...] += _nn(otb16, dhb)

    def edge_steps(u):
        return attn_fwd(jnp.where(u < 0, NB, 0), (u + QB * G) // G % QB, (u + G) % G, True)

    def head(b, c):
        st = edge_steps(b - 1)
        parts = iter((st[0:2], st[2:4], st[4:6], st[6:8]))

        def side():
            for x in next(parts):
                x()
        p1(b, side)
        return c
    lax.fori_loop(0, NB, head, 0)

    def f_edge(u, c):
        for st in edge_steps(u):
            st()
        return c
    lax.fori_loop(QB * G - 1, QB * G + jnp.minimum(pl.program_id(0), 0), f_edge, 0)

    for c in ins[3:]:
        c.wait()

    def p5(b):
        r0 = pl.multiple_of(b * T, T)
        dyt = jnp.zeros((D, T), F32)
        zs = []
        for i, ts in enumerate((dqt_s, dkt_s, dvt_s)):
            off = 0 if i == 0 else W // 128
            zt = jnp.concatenate(
                [jnp.concatenate([ts[g, b * QB + j + off] for j in range(QB)], 1)
                 for g in range(G)], 0)
            if i == 0:
                zt = zt * 0.25
            zt = zt.astype(BF16)
            zs.append(zt)
            dyt = dyt + _nn(wqkv_ref[:, i * D:(i + 1) * D], zt)
        y, r = _ln(x_ref[pl.ds(r0, T)].astype(F32))
        yt = y.T.astype(BF16)
        dy = dyt.T
        awqkv[:, 0:D] += _nt(yt, zs[0])
        dx_ref[pl.ds(r0, T)] = (dh_s[pl.ds(r0, T)] + _ln_bwd(dy, y, r)).astype(BF16)
        awqkv[:, D:2 * D] += _nt(yt, zs[1])
        awqkv[:, 2 * D:] += _nt(yt, zs[2])

    def blk(b, c):
        mlp(b)

        u = [attn_bwd(b, n // G, n % G) for n in range(QB * G)]
        for n in range(4 * QB * G + 2):
            for stage, lag in BWD_ORDER:
                m = n - lag
                if 0 <= m < 4 * QB * G:
                    u[m // 4][stage](m % 4)
        row_copy(0, b).start()
        return c
    lax.fori_loop(0, NB, blk, 0)
    for o, a in ((dwg_ref, awg), (dwu_ref, awu), (dwd_ref, awd), (dwo_ref, awo)):
        o[...] = a[...].astype(BF16)
    for c in outs[:4]:
        c.start()

    def tail(b, c):
        p5(b)
        row_copy(1, b).start()
        return c
    lax.fori_loop(0, NB, tail, 0)
    dwqkv_ref[...] = awqkv[...].astype(BF16)
    outs[4].start()
    for c in outs:
        c.wait()
    for k in range(2):
        for b in range(NB):
            row_copy(k, b).wait()


@jax.jit
def pallas_sequential_preLN__sliding_block__glu_gated_glu__prompt_kernel(
    A_x: jax.Array,
    A_wqkv: jax.Array,
    A_wo: jax.Array,
    B_x: jax.Array,
    B_w_gate: jax.Array,
    B_w_up: jax.Array,
    B_w_down: jax.Array,
    grad_out: jax.Array,
):
    V = pltpu.VMEM

    def P(shape):
        return V(shape[:-2] + (shape[-2] // 2, shape[-1]), jnp.int32)
    NK = (S + W) // 128 + 0
    scratch = [
        V((S, D), BF16), V((D, 3 * D), BF16), V((D, D), BF16), V((F, D), BF16), V((F, D), BF16),
        V((F, D), BF16), V((S, D), BF16),
        V((S, D), BF16), V((S, D), BF16), V((D, 3 * D), BF16), V((D, D), BF16), V((F, D), BF16),
        V((F, D), BF16), V((F, D), BF16),
        pltpu.SemaphoreType.DMA((8,)), pltpu.SemaphoreType.DMA((5,)), pltpu.SemaphoreType.DMA((2, NB)),
                P((G, S + W, 128)), P((G, S + 2 * W, 128)), P((G, S + 2 * W, 128)),
        V((G, S // 128, 128, 128), F32), P((G, NK + 2, 128, 128)), P((G, NK + 2, 128, 128)),
        P((2 * QB, G, 8, 320, 128)), V((NK, G, 8, 128), F32), V((G, NK, 128, 128), F32),
        P((G, T, 128)), V((G, QB, 128, 128), F32), V((G, QB, 8, 128), F32),
        V((S, D), F32),
        V((G, S // 128, 128, 128), F32), V((G, NK, 128, 128), F32), V((G, NK, 128, 128), F32),
        V((D, 3 * D), F32), V((D, D), F32), V((F, D), F32), V((F, D), F32), V((F, D), F32),
    ]
    sd = jax.ShapeDtypeStruct
    outs = pl.pallas_call(
        kernel,
        out_shape=(sd((S, D), BF16), sd((S, D), BF16), sd((D, 3 * D), BF16), sd((D, D), BF16),
                   sd((F, D), BF16), sd((F, D), BF16), sd((F, D), BF16)),
        in_specs=[pl.BlockSpec(memory_space=pl.ANY)] * 7,
        out_specs=[pl.BlockSpec(memory_space=pl.ANY)] * 7,
        grid=(1,),
        scratch_shapes=scratch,
        compiler_params=pltpu.CompilerParams(vmem_limit_bytes=120 * 1024 * 1024),
    )(A_x.reshape(S, D), A_wqkv, A_wo, B_w_gate.T, B_w_up.T, B_w_down, grad_out.reshape(S, D))
    return (outs[0].reshape(1, S, D), outs[1].reshape(1, S, D), outs[2], outs[3], outs[4].T, outs[5].T, outs[6])
```
